```python
import jax
import jax.numpy as jnp

def _softmax(x, axis=-1):
    return jax.nn.softmax(x, axis=axis)
def _gelu(x):
    return jax.nn.gelu(x, approximate=True)
def _silu(x):
    return jax.nn.silu(x)
def _sigmoid(x):
    return jax.nn.sigmoid(x)
def _layernorm(x, axis=-1, eps=1e-5):
    m = jnp.mean(x, axis=axis, keepdims=True)
    v = jnp.var(x, axis=axis, keepdims=True)
    return (x - m) / jnp.sqrt(v + eps)
def _scatter_add(tgt, idx, src, axis=0):
    return tgt.at[idx].add(src)
def _segment_sum(src, seg, n):
    return jax.ops.segment_sum(src, seg, n)
class _Rng:
    def __init__(self, key):
        self._k = key
    def _next(self):
        self._k, sub = jax.random.split(self._k)
        return sub
    def normal(self, shape):
        return jax.random.normal(self._next(), shape, dtype=jnp.bfloat16)
    def randint(self, lo, hi, shape):
        return jax.random.randint(self._next(), shape, lo, hi, dtype=jnp.int32)
    def uniform(self, shape, lo=0.0, hi=1.0):
        return jax.random.uniform(self._next(), shape, jnp.bfloat16, lo, hi)
    def permutation(self, n):
        return jax.random.permutation(self._next(), n)


kernel_name = 'standalone__qk_norm__prompt'

def setup_inputs():
    _rng = _Rng(jax.random.key(int.from_bytes(__import__("os").urandom(4), "little")))
    _w = (lambda a: (lambda t: t.astype(jnp.bfloat16) if jnp.issubdtype(t.dtype, jnp.floating) else t)(jnp.asarray(a)))
    B, H, S, D = 2, 32, 2048, 1024
    Dh = D // H
    return {
        "q": _w((lambda *s: _rng.normal(s) * 0.05)(B, H, S, Dh)),
        "k": _w((lambda *s: _rng.normal(s) * 0.05)(B, H, S, Dh)),
        "v": _w((lambda *s: _rng.normal(s) * 0.05)(B, H, S, Dh)),
        "t": _w(jnp.abs((lambda *s: _rng.normal(s) * 0.05)(H)) + 1.0),
    }

def reference(q, k, v, t):
    eps = 1e-6
    qn = q / (jnp.sqrt((q * q).sum(axis=-1, keepdims=True)) + eps)
    kn = k / (jnp.sqrt((k * k).sum(axis=-1, keepdims=True)) + eps)
    logits = jnp.einsum('bhqd,bhkd->bhqk', qn, kn) * t[None, :, None, None]
    attn = _softmax(logits, axis=-1)
    return jnp.einsum('bhqk,bhkd->bhqd', attn, v)
```

```python
import jax
import jax.numpy as jnp
from jax.experimental import pallas as pl
from jax.experimental.pallas import tpu as pltpu

LOG2E = 1.4426950408889634
EPS = 1e-6

BQ = 512
BK = 128
G = 2
BLAG = 1
TOK_LAG = 2
TOK_ROW = 64
PSZ = 512
STAGES = 4
K_OFF = 1
Q_OFF = 2
KT_N = 2
KT_OFF = 3


def _make_kernel(S, D, num_heads, heads_per_batch):
    NK = S // BK
    NQ = S // BQ
    NH = NQ * NK
    N = G * NH
    LAG = NK + BLAG
    assert S % BQ == 0 and S % PSZ == 0 and PSZ % BK == 0 and BQ % PSZ == 0
    assert NQ % 2 == 0 and BLAG >= 1 and BLAG < NK

    def i32(x):
        return pltpu.bitcast(x, jnp.int32)

    def kernel(t_ref, z_ref, q0_ref, k0_ref, *refs):
        qk_refs = refs[:2 * G]
        (v_ref, o_ref, kn_ref, qn_ref, s0_ref, s1_ref, acc_ref,
         mj0_ref, mcar_ref, kt_ref) = refs[2 * G:]
        step = pl.program_id(0)
        zero = z_ref[0]
        sbuf = (s0_ref, s1_ref)
        st = dict(m={}, mj={}, l={}, pb={}, s={}, tok={})

        def fold_or(z):
            out = z[0:8]
            for r in range(1, z.shape[0] // 8):
                out = out | z[r * 8:(r + 1) * 8]
            return out

        def norm_stages(src, dst, lo, hi, c):
            x = src[:, lo:hi].astype(jnp.float32)
            ss = jnp.sum(x * x, axis=0, keepdims=True)
            yield ss
            y = jnp.sqrt(ss) + EPS
            yield y
            inv = 1.0 / y
            if c is not None:
                inv = inv * c
            yield inv
            dst[:, lo:hi] = (x * inv).astype(jnp.bfloat16)
            yield fold_or(i32(dst[:, lo:hi]))

        def kt_stage():
            for u in range(KT_N):
                i = (LAG + u) % NK
                kt_ref[u] = kn_ref[:, i * BK:(i + 1) * BK].T
            yield fold_or(i32(kt_ref[KT_N - 1]))

        def pass_a(a, pre=None):
            T, i = divmod(a, NK)
            j = T % NQ
            qt = qn_ref[:, j * BQ:(j + 1) * BQ]
            if pre is not None:
                s = jnp.dot(kt_ref[pre], qt, preferred_element_type=jnp.float32)
            else:
                s = jax.lax.dot_general(
                    kn_ref[:, i * BK:(i + 1) * BK], qt, (((0,), (0,)), ((), ())),
                    preferred_element_type=jnp.float32)
            st["s"][a] = s
            sbuf[T % 2][i * BK:(i + 1) * BK, :] = s
            m = st["m"].get(T)
            for u in range(BK // 8):
                x = s[u * 8:(u + 1) * 8]
                m = x if m is None else jnp.maximum(m, x)
            st["m"][T] = m

        def tile_max(T):
            return jnp.broadcast_to(jnp.max(st["m"][T], axis=0, keepdims=True), (8, BQ))

        def pass_b(b):
            T, i = divmod(b, NK)
            if T not in st["mj"]:
                st["mj"][T] = mj0_ref[...] if T == 0 else tile_max(T)
            mj = st["mj"][T]
            at = b + LAG - TOK_LAG
            tok = None
            if at in st["s"] and not (T > 0 and at <= T * NK + NK - 1):
                tok = i32(st["s"][at][TOK_ROW:TOK_ROW + 8])
            for z in st["tok"].pop(b, []):
                if z.dtype != jnp.int32:
                    z = i32(jnp.broadcast_to(z, (8, z.shape[1])))
                if z.shape[1] < BQ:
                    z = jnp.concatenate([z] * (BQ // z.shape[1]), axis=1)
                tok = z if tok is None else tok | z
            if tok is not None:
                mj = pltpu.bitcast(i32(mj) | (tok & zero), jnp.float32)
            x = sbuf[T % 2][i * BK:(i + 1) * BK, :]
            p = jnp.exp2(x.reshape(BK // 8, 8, BQ) - mj[None]).reshape(BK, BQ)
            l = st["l"].get(T)
            for u in reversed(range(BK // 8)):
                y = p[u * 8:(u + 1) * 8]
                l = y if l is None else l + y
            st["l"][T] = l
            st["pb"][b] = p.astype(jnp.bfloat16)

        def pass_pv(b):
            T, i = divmod(b, NK)
            g, j = divmod(T, NQ)
            x = jnp.dot(v_ref[g, :, i * BK:(i + 1) * BK], st["pb"].pop(b),
                        preferred_element_type=jnp.float32)
            if i == 0:
                acc_ref[...] = x
            elif i < NK - 1:
                acc_ref[...] += x
            else:
                l = jnp.sum(st["l"][T], axis=0, keepdims=True)
                o_ref[g, :, j * BQ:(j + 1) * BQ] = (
                    (acc_ref[...] + x) * (1.0 / l)).astype(o_ref.dtype)

        def save_carry(t_done):
            mj0_ref[...] = tile_max(t_done)
            mcar_ref[...] = st["m"][t_done + 1]

        @pl.when(step == 0)
        def _():
            c0 = t_ref[0] * LOG2E
            for lo in range(0, S, PSZ):
                for _ in norm_stages(k0_ref, kn_ref, lo, lo + PSZ, None):
                    pass
            for lo in range(0, S, PSZ):
                for _ in norm_stages(q0_ref, qn_ref, lo, lo + PSZ, c0):
                    pass
            for a in range(LAG):
                pass_a(a)
            save_carry(0)
            for _ in kt_stage():
                pass
            for d in st.values():
                d.clear()

        st["m"][1] = mcar_ref[...]
        extra = {}
        for g in range(G):
            head = jnp.minimum(step * G + g + 1, num_heads - 1)
            c = t_ref[head % heads_per_batch] * LOG2E
            q_ref, k_ref = qk_refs[2 * g], qk_refs[2 * g + 1]
            base = g * NH
            pieces = []
            for lo in range(0, S, PSZ):
                a_free = base + (NQ - 1) * NK + (lo + PSZ - 1) // BK
                first = base + NH + lo // BK
                pieces.append((a_free + K_OFF, first,
                               norm_stages(k_ref, kn_ref, lo, lo + PSZ, None)))
            for lo in range(0, S, PSZ):
                a_free = base + (lo // BQ) * NK + NK - 1
                first = base + NH + (lo // BQ) * NK
                a_last = max(a_free, base + LAG + STAGES - 1) + Q_OFF
                pieces.append((a_last, first,
                               norm_stages(q_ref, qn_ref, lo, lo + PSZ, c)))
            for a_last, first, gen in pieces:
                assert a_last < first
                a_last = min(a_last, N + LAG - 1)
                for sidx in range(STAGES):
                    extra.setdefault(a_last - (STAGES - 1 - sidx), []).append(gen)
        kt_piece = ((LAG + KT_N - 1) % NK) * BK // PSZ
        a_k = ((G - 1) * NH + (NQ - 1) * NK
               + ((kt_piece + 1) * PSZ - 1) // BK + K_OFF)
        extra.setdefault(max(a_k + 1, LAG + KT_N) + KT_OFF, []).append(kt_stage())

        for n in range(N):
            a = n + LAG
            pass_a(a, n if n < KT_N else None)
            for gen in extra.get(a, []):
                st["tok"].setdefault(n, []).append(next(gen))
            pass_b(n)
            pass_pv(n)
        save_carry(G * NQ)

    return kernel


@jax.jit
def pallas_standalone__qk_norm__prompt_kernel(
    q: jax.Array,
    k: jax.Array,
    v: jax.Array,
    t: jax.Array,
):
    B, H, S, D = q.shape
    nh = B * H
    assert nh % G == 0
    qT = jnp.swapaxes(q, 2, 3).reshape(nh, D, S)
    kT = jnp.swapaxes(k, 2, 3).reshape(nh, D, S)
    vT = jnp.swapaxes(v, 2, 3).reshape(nh, D, S)

    def next_head(g):
        return pl.BlockSpec(
            (None, D, S), lambda i: (jnp.minimum(i * G + g + 1, nh - 1), 0, 0))

    first_head = pl.BlockSpec((None, D, S), lambda i: (0, 0, 0))
    heads = pl.BlockSpec((G, D, S), lambda i: (i, 0, 0))
    smem = pl.BlockSpec(memory_space=pltpu.SMEM)
    oT = pl.pallas_call(
        _make_kernel(S, D, nh, H),
        grid=(nh // G,),
        in_specs=([smem, smem, first_head, first_head]
                  + [next_head(g) for g in range(G) for _ in range(2)] + [heads]),
        out_specs=heads,
        out_shape=jax.ShapeDtypeStruct((nh, D, S), q.dtype),
        scratch_shapes=[
            pltpu.VMEM((D, S), jnp.bfloat16),
            pltpu.VMEM((D, S), jnp.bfloat16),
            pltpu.VMEM((S, BQ), jnp.float32),
            pltpu.VMEM((S, BQ), jnp.float32),
            pltpu.VMEM((D, BQ), jnp.float32),
            pltpu.VMEM((8, BQ), jnp.float32),
            pltpu.VMEM((8, BQ), jnp.float32),
            pltpu.VMEM((KT_N, BK, D), jnp.bfloat16),
        ],
        compiler_params=pltpu.CompilerParams(
            dimension_semantics=("arbitrary",),
            vmem_limit_bytes=64 * 1024 * 1024),
    )(t.astype(jnp.float32), jnp.zeros((1,), jnp.int32), qT, kT, *([qT, kT] * G), vT)
    return jnp.swapaxes(oT.reshape(B, H, D, S), 2, 3)
```

```python
import jax
import jax.numpy as jnp
from jax.experimental import pallas as pl
from jax.experimental.pallas import tpu as pltpu

LOG2E = 1.4426950408889634
EPS = 1e-6

BQ = 512
BK = 128
G = 3
GE = 1
BLAG = 1
TOK_LAG = 2
TOK_ROW = 112
STAGES = 4
STAGE_GAP = 2
K_OFF = 1
Q_OFF = (1, 1, 1, 3)
KT_N = 3
KT_OFF = 1
START_STEP = 4


def _make_kernel(S, D, nh, heads_per_batch):
    NK = S // BK
    NQ = S // BQ
    NH = NQ * NK
    LAG = NK + BLAG
    NIT = (nh - GE) // G
    assert S % BQ == 0 and BQ % BK == 0 and NQ == len(Q_OFF)
    assert NQ % 2 == 0 and 1 <= BLAG < NK and KT_N <= NK - BLAG
    assert (nh - GE) % G == 0 and 1 <= GE <= G and NIT >= 1
    assert heads_per_batch & (heads_per_batch - 1) == 0

    def i32(x):
        return pltpu.bitcast(x, jnp.int32)

    def b16(x):
        return pltpu.bitcast(x, jnp.bfloat16)

    def fold_or(z):
        out = z[0:8]
        for r in range(1, z.shape[0] // 8):
            out = out | z[r * 8:(r + 1) * 8]
        return out

    def kernel(t_ref, z_ref, q_hbm, k_hbm, v_hbm, o_hbm, inb, obuf, kn_ref, qn_ref,
               s0_ref, s1_ref, acc_ref, mj0_ref, mcar_ref, kt_ref, sem_i, sem_o):
        zero = z_ref[0]
        sbuf = (s0_ref, s1_ref)

        def in_copies(it, slot):
            cps = []
            for g in range(G):
                head = jnp.minimum(it * G + g + 1, nh - 1)
                cps.append(pltpu.make_async_copy(
                    k_hbm.at[head], inb.at[slot, g], sem_i.at[slot]))
                cps.append(pltpu.make_async_copy(
                    q_hbm.at[head], inb.at[slot, G + g], sem_i.at[slot]))
            cps.append(pltpu.make_async_copy(
                v_hbm.at[pl.ds(jnp.minimum(it * G, nh - G), G)],
                inb.at[slot, pl.ds(2 * G, G)], sem_i.at[slot]))
            return cps

        def in_wait(slot):
            pltpu.make_async_copy(inb.at[slot], inb.at[slot], sem_i.at[slot]).wait()

        def out_group(it, slot):
            return pltpu.make_async_copy(
                obuf.at[slot], o_hbm.at[pl.ds(jnp.maximum(it * G, 0), G)], sem_o)

        def norm_stages(src, dst, lo, hi, c):
            x = src[:, lo:hi].astype(jnp.float32)
            ss = jnp.sum(x * x, axis=0, keepdims=True)
            yield ss
            y = jnp.sqrt(ss) + EPS
            yield y
            inv = 1.0 / y
            if c is not None:
                inv = inv * c
            yield inv
            dst[:, lo:hi] = i32((x * inv).astype(jnp.bfloat16))
            yield fold_or(dst[:, lo:hi])

        def kt_stage():
            for u in range(KT_N):
                i = (LAG + u) % NK
                kt_ref[u] = b16(kn_ref[:, i * BK:(i + 1) * BK]).T
            yield fold_or(i32(kt_ref[KT_N - 1]))

        def new_state():
            return dict(m={}, mj={}, l={}, pb={}, s={}, tok={})

        def pass_a(st, a, pre=None):
            T, i = divmod(a, NK)
            j = T % NQ
            qt = b16(qn_ref[:, j * BQ:(j + 1) * BQ])
            if pre is not None:
                s = jnp.dot(kt_ref[pre], qt, preferred_element_type=jnp.float32)
            else:
                s = jax.lax.dot_general(
                    b16(kn_ref[:, i * BK:(i + 1) * BK]), qt, (((0,), (0,)), ((), ())),
                    preferred_element_type=jnp.float32)
            st["s"][a] = s
            sbuf[T % 2][i * BK:(i + 1) * BK, :] = s
            m = st["m"].get(T)
            for u in range(BK // 8):
                x = s[u * 8:(u + 1) * 8]
                m = x if m is None else jnp.maximum(m, x)
            st["m"][T] = m

        def tile_max(st, T):
            return jnp.broadcast_to(
                jnp.max(st["m"][T], axis=0, keepdims=True), (8, BQ))

        def pass_b(st, b):
            T, i = divmod(b, NK)
            if T not in st["mj"]:
                st["mj"][T] = mj0_ref[...] if T == 0 else tile_max(st, T)
            mj = st["mj"][T]
            at = b + LAG - TOK_LAG
            tok = None
            if at in st["s"] and not (T > 0 and at <= T * NK + NK - 1):
                tok = i32(st["s"][at][TOK_ROW:TOK_ROW + 8])
            for z in st["tok"].pop(b, []):
                if z.dtype != jnp.int32:
                    z = i32(jnp.broadcast_to(z, (8, z.shape[1])))
                while z.shape[1] < BQ:
                    z = jnp.concatenate([z] * (min(BQ, 4 * z.shape[1]) // z.shape[1]),
                                        axis=1)
                tok = z if tok is None else tok | z
            if tok is not None:
                mj = pltpu.bitcast(i32(mj) | (tok & zero), jnp.float32)
            x = sbuf[T % 2][i * BK:(i + 1) * BK, :]
            p = jnp.exp2(x.reshape(BK // 8, 8, BQ) - mj[None]).reshape(BK, BQ)
            l = st["l"].get(T)
            for u in reversed(range(BK // 8)):
                y = p[u * 8:(u + 1) * 8]
                l = y if l is None else l + y
            st["l"][T] = l
            st["pb"][b] = p.astype(jnp.bfloat16)

        def pass_pv(st, b, slot, voff):
            T, i = divmod(b, NK)
            g, j = divmod(T, NQ)
            x = jnp.dot(inb[slot, 2 * G + voff + g, :, i * BK:(i + 1) * BK],
                        st["pb"].pop(b), preferred_element_type=jnp.float32)
            if i == 0:
                acc_ref[...] = x
            elif i < NK - 1:
                acc_ref[...] += x
            else:
                l = jnp.sum(st["l"][T], axis=0, keepdims=True)
                obuf[slot, g, :, j * BQ:(j + 1) * BQ] = (
                    (acc_ref[...] + x) * (1.0 / l)).astype(obuf.dtype)

        def save_carry(st, t_done):
            mj0_ref[...] = tile_max(st, t_done)
            mcar_ref[...] = st["m"][t_done + 1]

        pltpu.make_async_copy(k_hbm.at[0], inb.at[1, 0], sem_i.at[1]).start()
        pltpu.make_async_copy(q_hbm.at[0], inb.at[1, 1], sem_i.at[1]).start()
        for cp in in_copies(0, 0):
            cp.start()
        obuf[1] = jnp.zeros(obuf.shape[1:], obuf.dtype)
        c0 = t_ref[0] * LOG2E
        pltpu.make_async_copy(inb.at[1, pl.ds(0, 2)], inb.at[1, pl.ds(0, 2)],
                              sem_i.at[1]).wait()
        for lo in range(0, S, BQ):
            for _ in norm_stages(inb.at[1, 0], kn_ref, lo, lo + BQ, None):
                pass
        for lo in range(0, S, BQ):
            for _ in norm_stages(inb.at[1, 1], qn_ref, lo, lo + BQ, c0):
                pass
        st0 = new_state()
        for a in range(LAG):
            pass_a(st0, a)
        save_carry(st0, 0)
        for _ in kt_stage():
            pass
        in_wait(0)

        def iteration(it, last):
            n_heads = GE if last else G
            n_steps = n_heads * NH
            slot = it & 1
            head0 = it * G
            voff = (G - GE) if last else 0
            st = new_state()
            st["m"][1] = mcar_ref[...]

            extra = {}
            for g in range(n_heads - 1 if last else n_heads):
                head = jnp.minimum(head0 + g + 1, nh - 1)
                c = t_ref[head & (heads_per_batch - 1)] * LOG2E
                base = g * NH
                pieces = []
                for lo in range(0, S, BQ):
                    a_free = base + (NQ - 1) * NK + (lo + BQ - 1) // BK
                    pieces.append((a_free + K_OFF, base + NH + lo // BK, norm_stages(
                        inb.at[slot, g], kn_ref, lo, lo + BQ, None)))
                for j in range(NQ):
                    a_free = base + j * NK + NK - 1
                    a_last = (max(a_free, base + LAG + (STAGES - 1) * STAGE_GAP)
                              + Q_OFF[j])
                    pieces.append((a_last, base + NH + j * NK, norm_stages(
                        inb.at[slot, G + g], qn_ref, j * BQ, (j + 1) * BQ, c)))
                for a_last, first_read, gen in pieces:
                    assert a_last < first_read
                    a_last = min(a_last, n_steps + LAG - 1)
                    for sidx in range(STAGES):
                        extra.setdefault(
                            a_last - (STAGES - 1 - sidx) * STAGE_GAP, []).append(gen)
            if not last:
                a_k = ((n_heads - 1) * NH + (NQ - 1) * NK
                       + (((LAG + KT_N - 1) % NK) * BK // BQ + 1) * (BQ // BK) - 1
                       + K_OFF)
                extra.setdefault(max(a_k + 1, LAG + KT_N) + KT_OFF, []).append(
                    kt_stage())

            pending = []
            for n in range(n_steps):
                a = n + LAG
                if not (last and a >= n_steps):
                    pass_a(st, a, n if n < KT_N else None)
                    for gen in extra.get(a, []):
                        st["tok"].setdefault(n, []).append(next(gen))
                pass_b(st, n)
                pass_pv(st, n, slot, voff)
                if n == START_STEP - 1:
                    if not last:
                        for cp in in_copies(it + 1, 1 - slot):
                            cp.start()
                    pending.append(out_group(it - 1, 1 - slot))
                    pending[-1].start()
                if last and (n + 1) % NK == 0:
                    g, j = divmod(n // NK, NQ)
                    if g == n_heads - 1:
                        lanes = pl.ds(j * BQ, BQ)
                        pending.append(pltpu.make_async_copy(
                            obuf.at[slot, g, :, lanes], o_hbm.at[head0 + g, :, lanes],
                            sem_o))
                        pending[-1].start()
                    elif j == NQ - 1:
                        pending.append(pltpu.make_async_copy(
                            obuf.at[slot, g], o_hbm.at[head0 + g], sem_o))
                        pending[-1].start()
            if not last:
                save_carry(st, n_heads * NQ)
                in_wait(1 - slot)
            for cp in pending:
                cp.wait()

        def body(it, carry):
            iteration(it, False)
            return carry

        jax.lax.fori_loop(0, NIT, body, 0)
        iteration(NIT, True)

    return kernel


@jax.jit
def pallas_standalone__qk_norm__prompt_kernel(
    q: jax.Array,
    k: jax.Array,
    v: jax.Array,
    t: jax.Array,
):
    B, H, S, D = q.shape
    nh = B * H
    qT = jnp.swapaxes(q, 2, 3).reshape(nh, D, S)
    kT = jnp.swapaxes(k, 2, 3).reshape(nh, D, S)
    vT = jnp.swapaxes(v, 2, 3).reshape(nh, D, S)
    smem = pl.BlockSpec(memory_space=pltpu.SMEM)
    hbm = pl.BlockSpec(memory_space=pl.ANY)
    oT = pl.pallas_call(
        _make_kernel(S, D, nh, H),
        in_specs=[smem, smem, hbm, hbm, hbm],
        out_specs=hbm,
        out_shape=jax.ShapeDtypeStruct((nh, D, S), q.dtype),
        scratch_shapes=[
            pltpu.VMEM((2, 3 * G, D, S), jnp.bfloat16),
            pltpu.VMEM((2, G, D, S), jnp.bfloat16),
            pltpu.VMEM((D // 2, S), jnp.int32),
            pltpu.VMEM((D // 2, S), jnp.int32),
            pltpu.VMEM((S, BQ), jnp.float32),
            pltpu.VMEM((S, BQ), jnp.float32),
            pltpu.VMEM((D, BQ), jnp.float32),
            pltpu.VMEM((8, BQ), jnp.float32),
            pltpu.VMEM((8, BQ), jnp.float32),
            pltpu.VMEM((KT_N, BK, D), jnp.bfloat16),
            pltpu.SemaphoreType.DMA((2,)),
            pltpu.SemaphoreType.DMA(()),
        ],
        compiler_params=pltpu.CompilerParams(vmem_limit_bytes=64 * 1024 * 1024),
    )(t.astype(jnp.float32), jnp.zeros((1,), jnp.int32), qT, kT, vT)
    return jnp.swapaxes(oT.reshape(B, H, D, S), 2, 3)
```

```python
import jax
import jax.numpy as jnp
from jax.experimental import pallas as pl
from jax.experimental.pallas import tpu as pltpu

LOG2E = 1.4426950408889634
EPS = 1e-6

BQ = 512
BK = 128
G = 3
GE = 1
BLAG = 1
TOK_LAG = 2
TOK_ROW = 96
STAGES = 4
STAGE_GAP = 2
K_OFF = 1
Q_OFF = (2, 1, 1, 3)
KT_N = 3
KT_OFF = 2
START_STEP = 8


def _make_kernel(S, D, nh, heads_per_batch):
    NK = S // BK
    NQ = S // BQ
    NH = NQ * NK
    LAG = NK + BLAG
    NIT = (nh - GE) // G
    assert S % BQ == 0 and BQ % BK == 0 and NQ == len(Q_OFF)
    assert NQ % 2 == 0 and 1 <= BLAG < NK and KT_N <= NK - BLAG
    assert (nh - GE) % G == 0 and 1 <= GE <= G and NIT >= 1
    assert heads_per_batch & (heads_per_batch - 1) == 0

    def i32(x):
        return pltpu.bitcast(x, jnp.int32)

    def b16(x):
        return pltpu.bitcast(x, jnp.bfloat16)

    def fold_or(z):
        out = z[0:8]
        for r in range(1, z.shape[0] // 8):
            out = out | z[r * 8:(r + 1) * 8]
        return out

    def kernel(t_ref, z_ref, q_hbm, k_hbm, v_hbm, o_hbm, inb, obuf, kn_ref, qn_ref,
               s0_ref, s1_ref, acc_ref, mj0_ref, mcar_ref, kt_ref, sem_i, sem_o):
        zero = z_ref[0]
        sbuf = (s0_ref, s1_ref)

        def in_copies(it, slot):
            cps = []
            for g in range(G):
                head = jnp.minimum(it * G + g + 1, nh - 1)
                cps.append(pltpu.make_async_copy(
                    k_hbm.at[head], inb.at[slot, g], sem_i.at[slot]))
                cps.append(pltpu.make_async_copy(
                    q_hbm.at[head], inb.at[slot, G + g], sem_i.at[slot]))
            cps.append(pltpu.make_async_copy(
                v_hbm.at[pl.ds(jnp.minimum(it * G, nh - G), G)],
                inb.at[slot, pl.ds(2 * G, G)], sem_i.at[slot]))
            return cps

        def in_wait(slot):
            pltpu.make_async_copy(inb.at[slot], inb.at[slot], sem_i.at[slot]).wait()

        def out_group(it, slot):
            return pltpu.make_async_copy(
                obuf.at[slot], o_hbm.at[pl.ds(jnp.maximum(it * G, 0), G)], sem_o)

        def norm_stages(src, dst, lo, hi, c):
            x = src[:, lo:hi].astype(jnp.float32)
            ss = jnp.sum(x * x, axis=0, keepdims=True)
            yield ss
            y = jnp.sqrt(ss) + EPS
            yield y
            inv = 1.0 / y
            if c is not None:
                inv = inv * c
            yield inv
            dst[:, lo:hi] = i32((x * inv).astype(jnp.bfloat16))
            yield fold_or(dst[:, lo:hi])

        def kt_stage():
            for u in range(KT_N):
                i = (LAG + u) % NK
                kt_ref[u] = b16(kn_ref[:, i * BK:(i + 1) * BK]).T
            yield fold_or(i32(kt_ref[KT_N - 1]))

        def new_state():
            return dict(m={}, mj={}, l={}, pb={}, s={}, tok={})

        def pass_a(st, a, pre=None):
            T, i = divmod(a, NK)
            j = T % NQ
            qt = b16(qn_ref[:, j * BQ:(j + 1) * BQ])
            if pre is not None:
                s = jnp.dot(kt_ref[pre], qt, preferred_element_type=jnp.float32)
            else:
                s = jax.lax.dot_general(
                    b16(kn_ref[:, i * BK:(i + 1) * BK]), qt, (((0,), (0,)), ((), ())),
                    preferred_element_type=jnp.float32)
            st["s"][a] = s
            sbuf[T % 2][i * BK:(i + 1) * BK, :] = s
            m = st["m"].get(T)
            for u in range(BK // 8):
                x = s[u * 8:(u + 1) * 8]
                m = x if m is None else jnp.maximum(m, x)
            st["m"][T] = m

        def tile_max(st, T):
            return jnp.broadcast_to(
                jnp.max(st["m"][T], axis=0, keepdims=True), (8, BQ))

        def pass_b(st, b):
            T, i = divmod(b, NK)
            if T not in st["mj"]:
                st["mj"][T] = mj0_ref[...] if T == 0 else tile_max(st, T)
            mj = st["mj"][T]
            at = b + LAG - TOK_LAG
            tok = None
            if at in st["s"] and not (T > 0 and at <= T * NK + NK - 1):
                tok = i32(st["s"][at][TOK_ROW:TOK_ROW + 8])
            for z in st["tok"].pop(b, []):
                if z.dtype != jnp.int32:
                    z = i32(jnp.broadcast_to(z, (8, z.shape[1])))
                while z.shape[1] < BQ:
                    z = jnp.concatenate([z] * (min(BQ, 4 * z.shape[1]) // z.shape[1]),
                                        axis=1)
                tok = z if tok is None else tok | z
            if tok is not None:
                mj = pltpu.bitcast(i32(mj) | (tok & zero), jnp.float32)
            x = sbuf[T % 2][i * BK:(i + 1) * BK, :]
            p = jnp.exp2(x.reshape(BK // 8, 8, BQ) - mj[None]).reshape(BK, BQ)
            l = st["l"].get(T)
            for u in reversed(range(BK // 8)):
                y = p[u * 8:(u + 1) * 8]
                l = y if l is None else l + y
            st["l"][T] = l
            st["pb"][b] = p.astype(jnp.bfloat16)

        def pass_pv(st, b, slot, voff):
            T, i = divmod(b, NK)
            g, j = divmod(T, NQ)
            x = jnp.dot(inb[slot, 2 * G + voff + g, :, i * BK:(i + 1) * BK],
                        st["pb"].pop(b), preferred_element_type=jnp.float32)
            if i == 0:
                acc_ref[...] = x
            elif i < NK - 1:
                acc_ref[...] += x
            else:
                l = jnp.sum(st["l"][T], axis=0, keepdims=True)
                obuf[slot, g, :, j * BQ:(j + 1) * BQ] = (
                    (acc_ref[...] + x) * (1.0 / l)).astype(obuf.dtype)

        def save_carry(st, t_done):
            mj0_ref[...] = tile_max(st, t_done)
            mcar_ref[...] = st["m"][t_done + 1]

        pltpu.make_async_copy(k_hbm.at[0], inb.at[1, 0], sem_i.at[1]).start()
        pltpu.make_async_copy(q_hbm.at[0], inb.at[1, 1], sem_i.at[1]).start()
        for cp in in_copies(0, 0):
            cp.start()
        obuf[1] = jnp.zeros(obuf.shape[1:], obuf.dtype)
        c0 = t_ref[0] * LOG2E
        pltpu.make_async_copy(inb.at[1, pl.ds(0, 2)], inb.at[1, pl.ds(0, 2)],
                              sem_i.at[1]).wait()
        for lo in range(0, S, BQ):
            for _ in norm_stages(inb.at[1, 0], kn_ref, lo, lo + BQ, None):
                pass
        for lo in range(0, S, BQ):
            for _ in norm_stages(inb.at[1, 1], qn_ref, lo, lo + BQ, c0):
                pass
        st0 = new_state()
        for a in range(LAG):
            pass_a(st0, a)
        save_carry(st0, 0)
        for _ in kt_stage():
            pass
        for cp in in_copies(1, 1):
            cp.start()
        in_wait(0)

        def iteration(it, last):
            n_heads = GE if last else G
            n_steps = n_heads * NH
            slot = it & 1
            head0 = it * G
            voff = (G - GE) if last else 0
            st = new_state()
            st["m"][1] = mcar_ref[...]

            extra = {}
            for g in range(n_heads - 1 if last else n_heads):
                head = jnp.minimum(head0 + g + 1, nh - 1)
                c = t_ref[head & (heads_per_batch - 1)] * LOG2E
                base = g * NH
                pieces = []
                for lo in range(0, S, BQ):
                    a_free = base + (NQ - 1) * NK + (lo + BQ - 1) // BK
                    pieces.append((a_free + K_OFF, base + NH + lo // BK, norm_stages(
                        inb.at[slot, g], kn_ref, lo, lo + BQ, None)))
                for j in range(NQ):
                    a_free = base + j * NK + NK - 1
                    a_last = (max(a_free, base + LAG + (STAGES - 1) * STAGE_GAP)
                              + Q_OFF[j])
                    pieces.append((a_last, base + NH + j * NK, norm_stages(
                        inb.at[slot, G + g], qn_ref, j * BQ, (j + 1) * BQ, c)))
                for a_last, first_read, gen in pieces:
                    assert a_last < first_read
                    a_last = min(a_last, n_steps + LAG - 1)
                    for sidx in range(STAGES):
                        extra.setdefault(
                            a_last - (STAGES - 1 - sidx) * STAGE_GAP, []).append(gen)
            if not last:
                a_k = ((n_heads - 1) * NH + (NQ - 1) * NK
                       + (((LAG + KT_N - 1) % NK) * BK // BQ + 1) * (BQ // BK) - 1
                       + K_OFF)
                extra.setdefault(max(a_k + 1, LAG + KT_N) + KT_OFF, []).append(
                    kt_stage())

            pending = []
            for n in range(n_steps):
                a = n + LAG
                if not (last and a >= n_steps):
                    pass_a(st, a, n if n < KT_N else None)
                    for gen in extra.get(a, []):
                        st["tok"].setdefault(n, []).append(next(gen))
                pass_b(st, n)
                pass_pv(st, n, slot, voff)
                if n == START_STEP - 1:
                    pending.append(out_group(it - 1, 1 - slot))
                    pending[-1].start()
                if last and (n + 1) % NK == 0:
                    g, j = divmod(n // NK, NQ)
                    if g == n_heads - 1:
                        lanes = pl.ds(j * BQ, BQ)
                        pending.append(pltpu.make_async_copy(
                            obuf.at[slot, g, :, lanes], o_hbm.at[head0 + g, :, lanes],
                            sem_o))
                        pending[-1].start()
                    elif j == NQ - 1:
                        pending.append(pltpu.make_async_copy(
                            obuf.at[slot, g], o_hbm.at[head0 + g], sem_o))
                        pending[-1].start()
            if not last:
                save_carry(st, n_heads * NQ)
                for cp in in_copies(it + 2, slot):
                    cp.start()
            in_wait(1 - slot)
            for cp in pending:
                cp.wait()

        def body(it, carry):
            iteration(it, False)
            return carry

        jax.lax.fori_loop(0, NIT, body, 0)
        iteration(NIT, True)

    return kernel


@jax.jit
def pallas_standalone__qk_norm__prompt_kernel(
    q: jax.Array,
    k: jax.Array,
    v: jax.Array,
    t: jax.Array,
):
    B, H, S, D = q.shape
    nh = B * H
    qT = jnp.swapaxes(q, 2, 3).reshape(nh, D, S)
    kT = jnp.swapaxes(k, 2, 3).reshape(nh, D, S)
    vT = jnp.swapaxes(v, 2, 3).reshape(nh, D, S)
    smem = pl.BlockSpec(memory_space=pltpu.SMEM)
    hbm = pl.BlockSpec(memory_space=pl.ANY)
    oT = pl.pallas_call(
        _make_kernel(S, D, nh, H),
        in_specs=[smem, smem, hbm, hbm, hbm],
        out_specs=hbm,
        out_shape=jax.ShapeDtypeStruct((nh, D, S), q.dtype),
        scratch_shapes=[
            pltpu.VMEM((2, 3 * G, D, S), jnp.bfloat16),
            pltpu.VMEM((2, G, D, S), jnp.bfloat16),
            pltpu.VMEM((D // 2, S), jnp.int32),
            pltpu.VMEM((D // 2, S), jnp.int32),
            pltpu.VMEM((S, BQ), jnp.float32),
            pltpu.VMEM((S, BQ), jnp.float32),
            pltpu.VMEM((D, BQ), jnp.float32),
            pltpu.VMEM((8, BQ), jnp.float32),
            pltpu.VMEM((8, BQ), jnp.float32),
            pltpu.VMEM((KT_N, BK, D), jnp.bfloat16),
            pltpu.SemaphoreType.DMA((2,)),
            pltpu.SemaphoreType.DMA(()),
        ],
        compiler_params=pltpu.CompilerParams(vmem_limit_bytes=64 * 1024 * 1024),
    )(t.astype(jnp.float32), jnp.zeros((1,), jnp.int32), qT, kT, vT)
    return jnp.swapaxes(oT.reshape(B, H, D, S), 2, 3)
```
